```python
import jax
import jax.numpy as jnp

def _softmax(x, axis=-1):
    return jax.nn.softmax(x, axis=axis)
def _gelu(x):
    return jax.nn.gelu(x, approximate=True)
def _silu(x):
    return jax.nn.silu(x)
def _sigmoid(x):
    return jax.nn.sigmoid(x)
def _layernorm(x, axis=-1, eps=1e-5):
    m = jnp.mean(x, axis=axis, keepdims=True)
    v = jnp.var(x, axis=axis, keepdims=True)
    return (x - m) / jnp.sqrt(v + eps)
def _scatter_add(tgt, idx, src, axis=0):
    return tgt.at[idx].add(src)
def _segment_sum(src, seg, n):
    return jax.ops.segment_sum(src, seg, n)
class _Rng:
    def __init__(self, key):
        self._k = key
    def _next(self):
        self._k, sub = jax.random.split(self._k)
        return sub
    def normal(self, shape):
        return jax.random.normal(self._next(), shape, dtype=jnp.bfloat16)
    def randint(self, lo, hi, shape):
        return jax.random.randint(self._next(), shape, lo, hi, dtype=jnp.int32)
    def uniform(self, shape, lo=0.0, hi=1.0):
        return jax.random.uniform(self._next(), shape, jnp.bfloat16, lo, hi)
    def permutation(self, n):
        return jax.random.permutation(self._next(), n)


kernel_name = 'recurrent_scan__sliding_local_dilated__glu_gated_swiglu__prompt'

def setup_inputs():
    _rng = _Rng(jax.random.key(int.from_bytes(__import__("os").urandom(4), "little")))
    _w = (lambda a: (lambda t: t.astype(jnp.bfloat16) if jnp.issubdtype(t.dtype, jnp.floating) else t)(jnp.asarray(a)))
    def _A_setup():
        B, S, D = 1, 2048, 1024
        return {
            "x": _w((lambda *s: _rng.normal(s) * 0.05)(B, S, D)),
            "wqkv": _w((lambda *s: _rng.normal(s) * 0.05)(D, 3 * D)),
            "wo": _w((lambda *s: _rng.normal(s) * 0.05)(D, D)),
        }
    _A_in = _A_setup()

    def _B_setup():
        B, S, D, F = 1, 2048, 1024, 3584
        return {
            "x": _w((lambda *s: _rng.normal(s) * 0.05)(B, S, D)),
            "w1": _w((lambda *s: _rng.normal(s) * 0.05)(D, F) * (2.0 / D) ** 0.5),
            "w3": _w((lambda *s: _rng.normal(s) * 0.05)(D, F) * (2.0 / D) ** 0.5),
            "w2": _w((lambda *s: _rng.normal(s) * 0.05)(F, D) * (2.0 / F) ** 0.5),
        }
    _B_in = _B_setup()

    return {
        "A_x": _A_in["x"],
        "A_wqkv": _A_in["wqkv"],
        "A_wo": _A_in["wo"],
        "B_x": _B_in["x"],
        "B_w1": _B_in["w1"],
        "B_w3": _B_in["w3"],
        "B_w2": _B_in["w2"],
    }

def reference(A_x, A_wqkv, A_wo, B_x, B_w1, B_w3, B_w2):
    def _A_ref(x, wqkv, wo):
        B, S, D = x.shape
        H = 32; Dh = D // H
        W, dil = 8, 2
        qkv = (lambda x, *d: x.transpose(*d))((x @ wqkv).reshape(B, S, 3, H, Dh), 2, 0, 3, 1, 4)
        q, k, v = qkv[0], qkv[1], qkv[2]
        scale = Dh ** -0.5
        pos = jnp.arange(S)
        off = jnp.arange(W) * dil
        idx = pos[:, None] - off[None, :]
        mask = idx >= 0
        idx_c = jnp.where(mask, idx, 0).reshape(-1)
        kg = k[:, :, idx_c, :].reshape(B, H, S, W, Dh)
        vg = v[:, :, idx_c, :].reshape(B, H, S, W, Dh)
        logits = jnp.einsum("bhsd,bhswd->bhsw", q, kg) * scale
        logits = jnp.where(mask[None, None, :, :], logits, -1e9)
        attn = _softmax(logits, axis=-1)
        o = jnp.einsum("bhsw,bhswd->bhsd", attn, vg)
        return (lambda x, *d: x.transpose(*d))(o, 0, 2, 1, 3).reshape(B, S, D) @ wo

    def _B_ref(x, w1, w3, w2):
        gate = jnp.einsum("bsd,df->bsf", x, w1)
        up = jnp.einsum("bsd,df->bsf", x, w3)
        h = _silu(gate) * up
        out = jnp.einsum("bsf,fd->bsd", h, w2)
        return out

    x = A_x
    xn = _layernorm(x, axis=-1)
    s = _A_ref(xn, A_wqkv, A_wo)
    g = _silu(_B_ref(xn, B_w1, B_w3, B_w2))
    return x + s * g
```

```python
import functools
import math
import jax
import jax.numpy as jnp
from jax import lax
import jax.experimental.pallas as pl
import jax.experimental.pallas.tpu as pltpu

S, D, F = 2048, 1024, 3584
H, DH, W, DIL = 32, 32, 8, 2
HALO = 16
NC = D // 128
BF = jnp.bfloat16
F32 = jnp.float32


def swap8(xs):
    xs = list(xs)
    lane = lax.broadcasted_iota(jnp.int32, xs[0].shape, 1)
    for b in range(3):
        s = 4 << b
        m = (lane & s) == 0
        for c in range(NC):
            if c & (1 << b):
                continue
            a, bb = xs[c], xs[c | (1 << b)]
            xs[c] = jnp.where(m, a, pltpu.roll(bb, s, 1))
            xs[c | (1 << b)] = jnp.where(m, pltpu.roll(a, 128 - s, 1), bb)
    return xs


def make(T=512, N2=4, N3=4, MS=512, attn_pos="after", packed=True, SB=8, RB=8, OB=16):
    NT = S // T
    FC = F // N2
    NO = D // N3
    R2 = T // N2
    R3 = T // N3
    EXPC = (DH ** -0.5) * math.log2(math.e)

    def layernorm(xb):
        x = xb.astype(F32)
        m = jnp.mean(x, axis=-1, keepdims=True)
        xc = x - m
        var = jnp.mean(xc * xc, axis=-1, keepdims=True)
        return (xc * lax.rsqrt(var + 1e-5)).astype(BF)

    def mm(a_ref_fn, b):
        outs = [jnp.dot(a_ref_fn(r0, r0 + MS), b, preferred_element_type=F32) for r0 in range(0, T, MS)]
        return outs[0] if len(outs) == 1 else jnp.concatenate(outs, axis=0)

    def kernel(x_hbm, wqkv_hbm, wo_hbm, w1_hbm, w3_hbm, w2_hbm, out_hbm,
               wq_s, w1_s, w3_s, w2_s, wo_s, x_s, xn_s, raw_q, raw_k, raw_v,
               q_s, k_s, v_s, o_s, ob_s, h_s, st_s, wsem, osem):
        i = pl.program_id(0)
        slot = i % 2

        def cp_qkv(t):
            return pltpu.make_async_copy(wqkv_hbm.at[:, t * D:(t + 1) * D], wq_s.at[t], wsem.at[t])

        def cp_w1(c):
            return pltpu.make_async_copy(w1_hbm.at[:, pl.ds(c * FC, FC)], w1_s.at[c], wsem.at[3 + c])

        def cp_w3(c):
            return pltpu.make_async_copy(w3_hbm.at[:, pl.ds(c * FC, FC)], w3_s.at[c], wsem.at[3 + N2 + c])

        def cp_w2(n):
            return pltpu.make_async_copy(w2_hbm.at[:, pl.ds(n * NO, NO)], w2_s.at[n], wsem.at[3 + 2 * N2 + n])

        def cp_wo(n):
            return pltpu.make_async_copy(wo_hbm.at[:, pl.ds(n * NO, NO)], wo_s.at[n], wsem.at[3 + 2 * N2 + N3 + n])

        def cp_x(t):
            return pltpu.make_async_copy(x_hbm.at[pl.ds(t * T, T), :], x_s.at[t], wsem.at[3 + 2 * N2 + 2 * N3 + t])

        def cp_out(n):
            return pltpu.make_async_copy(st_s.at[n], out_hbm.at[pl.ds(i * T, T), pl.ds(n * NO, NO)], osem.at[n])

        @pl.when(i == 0)
        def _():
            cp_x(0).start()
            for t in range(3):
                cp_qkv(t).start()
            for c in range(N2):
                cp_w1(c).start()
                cp_w3(c).start()
            for n in range(N3):
                cp_w2(n).start()
                cp_wo(n).start()
            for t in range(1, NT):
                cp_x(t).start()
            k_s[:, T:T + HALO, :] = jnp.zeros((NC, HALO, 128), F32)
            v_s[:, T:T + HALO, :] = jnp.zeros((NC, HALO, 128), F32)
            cp_x(0).wait()
            for r0 in range(0, T, 128):
                xn_s[0, r0:r0 + 128, :] = layernorm(x_s[0, r0:r0 + 128, :])
            cp_qkv(0).wait()

        def lhs(r0, r1):
            return xn_s[slot, r0:r1, :]

        def swap_rows(src, dst, off, base, nrows):
            if not packed:
                for r0 in range(0, nrows, SB):
                    ys = swap8([src[pl.ds(base + r0, SB), c * 128:(c + 1) * 128] for c in range(NC)])
                    for c in range(NC):
                        dst[c, pl.ds(off + base + r0, SB), :] = ys[c]
                return
            for r0 in range(0, nrows, 2 * SB):
                ps = [pltpu.pack_elementwise(
                    [src[pl.ds(base + r0, SB), c * 128:(c + 1) * 128],
                     src[pl.ds(base + r0 + SB, SB), c * 128:(c + 1) * 128]], packed_dtype=BF) for c in range(NC)]
                ys = swap8(ps)
                for c in range(NC):
                    dst[c, pl.ds(off + base + r0, SB), :] = pltpu.unpack_elementwise(
                        ys[c], index=0, packed_dtype=BF, unpacked_dtype=F32)
                    dst[c, pl.ds(off + base + r0 + SB, SB), :] = pltpu.unpack_elementwise(
                        ys[c], index=1, packed_dtype=BF, unpacked_dtype=F32)

        k_s[:, 0:HALO, :] = k_s[:, T:T + HALO, :]
        v_s[:, 0:HALO, :] = v_s[:, T:T + HALO, :]
        raw_q[...] = mm(lhs, wq_s[0])

        @pl.when(i == 0)
        def _():
            cp_qkv(1).wait()

        raw_k[...] = mm(lhs, wq_s[1])
        swap_rows(raw_q, q_s, 0, 0, T)

        @pl.when(i == 0)
        def _():
            cp_qkv(2).wait()

        raw_v[...] = mm(lhs, wq_s[2])
        swap_rows(raw_k, k_s, HALO, 0, T)

        def attn_group(base, r0):
            rb = base + r0
            qs = [q_s[c, pl.ds(rb, RB), :] for c in range(NC)]
            lane = lax.broadcasted_iota(jnp.int32, (RB, 128), 1)
            b0 = (lane & 1) == 0
            b1 = (lane & 2) == 0
            logits = []
            for j in range(W):
                st = HALO + rb - DIL * j
                acc = qs[0] * k_s[0, pl.ds(st, RB), :]
                for c in range(1, NC):
                    acc = acc + qs[c] * k_s[c, pl.ds(st, RB), :]
                logits.append(acc)
            logits = [acc + jnp.where(b0, pltpu.roll(acc, 127, 1), pltpu.roll(acc, 1, 1)) for acc in logits]
            logits = [acc + jnp.where(b1, pltpu.roll(acc, 126, 1), pltpu.roll(acc, 2, 1)) for acc in logits]
            if r0 < HALO:
                row = i * T + rb + lax.broadcasted_iota(jnp.int32, (RB, 128), 0)
                logits = [logits[0]] + [jnp.where(row >= DIL * j, logits[j], -1e9) for j in range(1, W)]
            mx = logits[0]
            for j in range(1, W):
                mx = jnp.maximum(mx, logits[j])
            es = [jnp.exp2((l - mx) * EXPC) for l in logits]
            den = es[0]
            for j in range(1, W):
                den = den + es[j]
            inv = 1.0 / den
            ps = [e * inv for e in es]
            for c in range(NC):
                acc = None
                for j in range(W):
                    st = HALO + rb - DIL * j
                    t = ps[j] * v_s[c, pl.ds(st, RB), :]
                    acc = t if acc is None else acc + t
                o_s[c, r0:r0 + RB, :] = acc

        def p2(c, carry):
            @pl.when(i == 0)
            def _():
                cp_w1(c).wait()
                cp_w3(c).wait()

            base = pl.multiple_of(c * R2, R2)

            def attn():
                swap_rows(raw_v, v_s, HALO, base, R2)
                for r0 in range(0, R2, RB):
                    attn_group(base, r0)
                for r0 in range(0, R2, OB):
                    ts = [pltpu.bitcast(o_s[cc, r0:r0 + OB, :].astype(BF), jnp.uint32) for cc in range(NC)]
                    ts = swap8(ts)
                    for cc in range(NC):
                        ob_s[pl.ds(base + r0, OB), cc * 128:(cc + 1) * 128] = pltpu.bitcast(ts[cc], BF)

            if attn_pos == "before":
                attn()
            g = mm(lhs, w1_s[c])
            u = mm(lhs, w3_s[c])
            h_s[c] = (g * jax.nn.sigmoid(g) * u).astype(BF)
            if attn_pos == "after":
                attn()
            return carry

        lax.fori_loop(0, N2, p2, 0)

        nxt = jnp.minimum(i + 1, NT - 1)

        def p3(n, carry):
            @pl.when(i == 0)
            def _():
                cp_w2(n).wait()
                cp_wo(n).wait()

            @pl.when(i > 0)
            def _():
                cp_out(n).wait()

            @pl.when(jnp.logical_and(n == 0, i + 1 < NT))
            def _():
                cp_x(i + 1).wait()

            f = None
            for c in range(N2):
                t = mm(lambda r0, r1: h_s[c, r0:r1, :], w2_s[n, c * FC:(c + 1) * FC, :])
                f = t if f is None else f + t
            s = mm(lambda r0, r1: ob_s[r0:r1, :], wo_s[n])
            gg = f * jax.nn.sigmoid(f)
            xr = x_s[i, :, pl.ds(pl.multiple_of(n * NO, NO), NO)].astype(F32)
            st_s[n] = (xr + s * gg).astype(BF)
            cp_out(n).start()
            rb = pl.multiple_of(n * R3, R3)
            for r0 in range(0, R3, 128):
                xn_s[1 - slot, pl.ds(rb + r0, 128), :] = layernorm(x_s[nxt, pl.ds(rb + r0, 128), :])
            return carry

        lax.fori_loop(0, N3, p3, 0)

        @pl.when(i == NT - 1)
        def _():
            for n in range(N3):
                cp_out(n).wait()

    any_spec = pl.BlockSpec(memory_space=pl.ANY)

    @jax.jit
    def run(x, wqkv, wo, w1, w3, w2):
        return pl.pallas_call(
            kernel,
            grid=(NT,),
            in_specs=[any_spec] * 6,
            out_specs=any_spec,
            out_shape=jax.ShapeDtypeStruct((S, D), BF),
            scratch_shapes=[pltpu.VMEM((3, D, D), BF),
                            pltpu.VMEM((N2, D, FC), BF),
                            pltpu.VMEM((N2, D, FC), BF),
                            pltpu.VMEM((N3, F, NO), BF),
                            pltpu.VMEM((N3, D, NO), BF),
                            pltpu.VMEM((NT, T, D), BF),
                            pltpu.VMEM((2, T, D), BF),
                            pltpu.VMEM((T, D), F32),
                            pltpu.VMEM((T, D), F32),
                            pltpu.VMEM((T, D), F32),
                            pltpu.VMEM((NC, T, 128), F32),
                            pltpu.VMEM((NC, T + HALO, 128), F32),
                            pltpu.VMEM((NC, T + HALO, 128), F32),
                            pltpu.VMEM((NC, R2, 128), F32),
                            pltpu.VMEM((T, D), BF),
                            pltpu.VMEM((N2, T, FC), BF),
                            pltpu.VMEM((N3, T, NO), BF),
                            pltpu.SemaphoreType.DMA((3 + 2 * N2 + 2 * N3 + NT,)),
                            pltpu.SemaphoreType.DMA((N3,))],
            compiler_params=pltpu.CompilerParams(dimension_semantics=("arbitrary",),
                                                 vmem_limit_bytes=110 * 1024 * 1024),
        )(x, wqkv, wo, w1, w3, w2)
    return run


_RUN = make(**{'RB':16,'SB':16,'OB':32})


@jax.jit
def pallas_recurrent_scan__sliding_local_dilated__glu_gated_swiglu__prompt_kernel(
    A_x: jax.Array,
    A_wqkv: jax.Array,
    A_wo: jax.Array,
    B_x: jax.Array,
    B_w1: jax.Array,
    B_w3: jax.Array,
    B_w2: jax.Array,
):
    del B_x
    out = _RUN(A_x.reshape(S, D), A_wqkv, A_wo, B_w1, B_w3, B_w2)
    return out.reshape(A_x.shape)
```

```python
import functools
import math
import jax
import jax.numpy as jnp
from jax import lax
import jax.experimental.pallas as pl
import jax.experimental.pallas.tpu as pltpu

S, D, F = 2048, 1024, 3584
H, DH, W, DIL = 32, 32, 8, 2
HALO = 16
NC = D // 128
BF = jnp.bfloat16
F32 = jnp.float32


def swap8(xs):
    xs = list(xs)
    lane = lax.broadcasted_iota(jnp.int32, xs[0].shape, 1)
    for b in range(3):
        s = 4 << b
        m = (lane & s) == 0
        for c in range(NC):
            if c & (1 << b):
                continue
            a, bb = xs[c], xs[c | (1 << b)]
            xs[c] = jnp.where(m, a, pltpu.roll(bb, s, 1))
            xs[c | (1 << b)] = jnp.where(m, pltpu.roll(a, 128 - s, 1), bb)
    return xs


def silu(x):
    a = 0.5 * x
    return a + a * jnp.tanh(a)


def ln_rows(x):
    m = jnp.mean(x, axis=-1, keepdims=True)
    xc = x - m
    var = jnp.mean(xc * xc, axis=-1, keepdims=True)
    return xc * lax.rsqrt(var + 1e-5)


def dot(a, b):
    return jnp.dot(a, b, preferred_element_type=F32)


def make(T=512, N2=2, N3=2, SB=16, RB=16, OB=32, chain=1, LNB=16, XSPLIT=(256, 256), QSPLIT=(256, 256, 512),
         OSPLIT=1, SUB=None, PMODE=0):
    NT = S // T
    FC = F // N2
    NO = D // N3
    R2 = T // N2
    R3 = T // N3
    EXPC = (DH ** -0.5) * math.log2(math.e)
    assert sum(XSPLIT) == T and sum(QSPLIT) == D
    xoff = [sum(XSPLIT[:k]) for k in range(len(XSPLIT) + 1)]
    qoff = [sum(QSPLIT[:k]) for k in range(len(QSPLIT) + 1)]
    SX0 = 0
    SQ = SX0 + len(XSPLIT)
    SKV = SQ + len(QSPLIT)
    SW1 = SKV + 2
    SW3 = SW1 + N2
    SW2 = SW3 + N2
    SWO = SW2 + N3
    SX = SWO + N3
    NSEM = SX + NT - 1
    OW = NO // OSPLIT

    def kernel(x_hbm, wqkv_hbm, wo_hbm, w1_hbm, w3_hbm, w2_hbm, out_hbm,
               wq_s, w1_s, w3_s, w2_s, wo_s, x_s, xn_s, raw,
               qkv_s, o_s, ob_s, h_s, st_s, wsem, osem):
        i = pl.program_id(0)
        slot = i % 2
        q_s, k_s, v_s = qkv_s.at[0], qkv_s.at[1], qkv_s.at[2]

        def cp_x0(k):
            return pltpu.make_async_copy(x_hbm.at[xoff[k]:xoff[k + 1], :], x_s.at[0, xoff[k]:xoff[k + 1], :],
                                         wsem.at[SX0 + k])

        def cp_q(k):
            return pltpu.make_async_copy(wqkv_hbm.at[:, qoff[k]:qoff[k + 1]], wq_s.at[0, :, qoff[k]:qoff[k + 1]],
                                         wsem.at[SQ + k])

        def cp_kv(t):
            return pltpu.make_async_copy(wqkv_hbm.at[:, pl.ds(t * D, D)], wq_s.at[t], wsem.at[SKV + t - 1])

        def cp_w1(c):
            return pltpu.make_async_copy(w1_hbm.at[:, pl.ds(c * FC, FC)], w1_s.at[c], wsem.at[SW1 + c])

        def cp_w3(c):
            return pltpu.make_async_copy(w3_hbm.at[:, pl.ds(c * FC, FC)], w3_s.at[c], wsem.at[SW3 + c])

        def cp_w2(n):
            return pltpu.make_async_copy(w2_hbm.at[:, pl.ds(n * NO, NO)], w2_s.at[n], wsem.at[SW2 + n])

        def cp_wo(n):
            return pltpu.make_async_copy(wo_hbm.at[:, pl.ds(n * NO, NO)], wo_s.at[n], wsem.at[SWO + n])

        def cp_x(t):
            return pltpu.make_async_copy(x_hbm.at[pl.ds(t * T, T), :], x_s.at[t], wsem.at[SX + t - 1])

        def cp_out(n, p):
            return pltpu.make_async_copy(st_s.at[n, p], out_hbm.at[pl.ds(i * T, T), pl.ds(n * NO + p * OW, OW)],
                                         osem.at[n * OSPLIT + p])

        @pl.when(i == 0)
        def _():
            nx, nq = len(XSPLIT), len(QSPLIT)
            if PMODE == 0:
                for k in range(max(nx, nq)):
                    if k < nx:
                        cp_x0(k).start()
                    if k < nq:
                        cp_q(k).start()
            else:
                for k in range(nx):
                    cp_x0(k).start()
                for k in range(nq):
                    cp_q(k).start()
            for t in (1, 2):
                cp_kv(t).start()
            for c in range(N2):
                cp_w1(c).start()
                cp_w3(c).start()
            for n in range(N3):
                cp_w2(n).start()
                cp_wo(n).start()
            for t in range(1, NT):
                cp_x(t).start()
            k_s[:, T:T + HALO, :] = jnp.zeros((NC, HALO, 128), F32)
            v_s[:, T:T + HALO, :] = jnp.zeros((NC, HALO, 128), F32)
            if PMODE == 0:
                for k in range(nx):
                    cp_x0(k).wait()
                    for r0 in range(xoff[k], xoff[k + 1], 128):
                        xn_s[0, r0:r0 + 128, :] = ln_rows(x_s[0, r0:r0 + 128, :].astype(F32)).astype(BF)
                    if k == 0:
                        cp_q(0).wait()
                    raw[0, xoff[k]:xoff[k + 1], qoff[0]:qoff[1]] = dot(xn_s[0, xoff[k]:xoff[k + 1], :],
                                                                       wq_s[0, :, qoff[0]:qoff[1]])
                kq0 = 1
            else:
                for k in range(nx):
                    cp_x0(k).wait()
                    for r0 in range(xoff[k], xoff[k + 1], 128):
                        xn_s[0, r0:r0 + 128, :] = ln_rows(x_s[0, r0:r0 + 128, :].astype(F32)).astype(BF)
                kq0 = 0
            for k in range(kq0, nq):
                cp_q(k).wait()
                raw[0, :, qoff[k]:qoff[k + 1]] = dot(xn_s[0], wq_s[0, :, qoff[k]:qoff[k + 1]])

        def swap_rows(src, dst, base, nrows):
            for r0 in range(0, nrows, 2 * SB):
                ps = [pltpu.pack_elementwise(
                    [src[pl.ds(base + r0, SB), c * 128:(c + 1) * 128],
                     src[pl.ds(base + r0 + SB, SB), c * 128:(c + 1) * 128]], packed_dtype=BF) for c in range(NC)]
                ys = swap8(ps)
                for c in range(NC):
                    dst[c, pl.ds(HALO + base + r0, SB), :] = pltpu.unpack_elementwise(
                        ys[c], index=0, packed_dtype=BF, unpacked_dtype=F32)
                    dst[c, pl.ds(HALO + base + r0 + SB, SB), :] = pltpu.unpack_elementwise(
                        ys[c], index=1, packed_dtype=BF, unpacked_dtype=F32)

        k_s[:, 0:HALO, :] = k_s[:, T:T + HALO, :]
        v_s[:, 0:HALO, :] = v_s[:, T:T + HALO, :]

        def pb(t, carry):
            @pl.when(i == 0)
            def _():
                cp_kv(t).wait()

            raw[t] = dot(xn_s[slot], wq_s[t])
            return carry

        lax.fori_loop(jnp.where(i == 0, 1, 0), 3, pb, 0)

        def attn_group(base, r0, dep):
            rb = base + r0
            qs = [q_s[c, pl.ds(HALO + rb, RB), :] for c in range(NC)]
            if dep is not None:
                qs[0] = jnp.where(i < 0, dep, qs[0])
            lane = lax.broadcasted_iota(jnp.int32, (RB, 128), 1)
            b0 = (lane & 1) == 0
            b1 = (lane & 2) == 0
            logits = []
            for j in range(W):
                st = HALO + rb - DIL * j
                acc = qs[0] * k_s[0, pl.ds(st, RB), :]
                for c in range(1, NC):
                    acc = acc + qs[c] * k_s[c, pl.ds(st, RB), :]
                logits.append(acc)
            logits = [acc + jnp.where(b0, pltpu.roll(acc, 127, 1), pltpu.roll(acc, 1, 1)) for acc in logits]
            logits = [acc + jnp.where(b1, pltpu.roll(acc, 126, 1), pltpu.roll(acc, 2, 1)) for acc in logits]
            if r0 < HALO:
                row = i * T + rb + lax.broadcasted_iota(jnp.int32, (RB, 128), 0)
                logits = [logits[0]] + [jnp.where(row >= DIL * j, logits[j], -1e9) for j in range(1, W)]
            mx = logits[0]
            for j in range(1, W):
                mx = jnp.maximum(mx, logits[j])
            es = [jnp.exp2((l - mx) * EXPC) for l in logits]
            den = es[0]
            for j in range(1, W):
                den = den + es[j]
            inv = 1.0 / den
            ps = [e * inv for e in es]
            for c in range(NC):
                acc = None
                for j in range(W):
                    st = HALO + rb - DIL * j
                    t = ps[j] * v_s[c, pl.ds(st, RB), :]
                    acc = t if acc is None else acc + t
                o_s[c, r0:r0 + RB, :] = acc
            return acc

        def p2(c, carry):
            @pl.when(i == 0)
            def _():
                cp_w1(c).wait()
                cp_w3(c).wait()

            base = pl.multiple_of(c * R2, R2)
            sub = SUB or FC
            for s0 in range(0, FC, sub):
                s1 = min(s0 + sub, FC)
                g = dot(xn_s[slot], w1_s[c, :, s0:s1])
                u = dot(xn_s[slot], w3_s[c, :, s0:s1])
                h_s[c, :, s0:s1] = (silu(g) * u).astype(BF)

            for t in range(3):
                swap_rows(raw.at[t], qkv_s.at[t], base, R2)
            outs = []
            for r0 in range(0, R2, RB):
                dep = outs[-chain] if chain and len(outs) >= chain else None
                outs.append(attn_group(base, r0, dep))
            for r0 in range(0, R2, OB):
                ts = [pltpu.bitcast(o_s[cc, r0:r0 + OB, :].astype(BF), jnp.uint32) for cc in range(NC)]
                ts = swap8(ts)
                for cc in range(NC):
                    ob_s[pl.ds(base + r0, OB), cc * 128:(cc + 1) * 128] = pltpu.bitcast(ts[cc], BF)
            return carry

        lax.fori_loop(0, N2, p2, 0)

        nxt = jnp.minimum(i + 1, NT - 1)

        def p3(n, carry):
            @pl.when(i == 0)
            def _():
                cp_w2(n).wait()
                cp_wo(n).wait()

            @pl.when(i > 0)
            def _():
                for p in range(OSPLIT):
                    cp_out(n, p).wait()

            @pl.when(jnp.logical_and(n == 0, i + 1 < NT))
            def _():
                cp_x(i + 1).wait()

            for p in range(OSPLIT):
                f = None
                for c in range(N2):
                    t = dot(h_s[c], w2_s[n, c * FC:(c + 1) * FC, p * OW:(p + 1) * OW])
                    f = t if f is None else f + t
                s = dot(ob_s[...], wo_s[n, :, p * OW:(p + 1) * OW])
                xr = x_s[i, :, pl.ds(pl.multiple_of(n * NO + p * OW, OW), OW)].astype(F32)
                st_s[n, p] = (xr + s * silu(f)).astype(BF)
                cp_out(n, p).start()

            rb = pl.multiple_of(n * R3, R3)
            prev = None
            for r0 in range(0, R3, LNB):
                xb = x_s[nxt, pl.ds(rb + r0, LNB), :].astype(F32)
                if prev is not None:
                    x0 = jnp.where(i < 0, prev, xb[:, 0:128])
                    xb = jnp.concatenate([x0, xb[:, 128:]], axis=1)
                y = ln_rows(xb)
                prev = y[:, 0:128]
                xn_s[1 - slot, pl.ds(rb + r0, LNB), :] = y.astype(BF)
            return carry

        lax.fori_loop(0, N3, p3, 0)

        @pl.when(i == NT - 1)
        def _():
            for n in range(N3):
                for p in range(OSPLIT):
                    cp_out(n, p).wait()

    any_spec = pl.BlockSpec(memory_space=pl.ANY)

    @jax.jit
    def run(x, wqkv, wo, w1, w3, w2):
        return pl.pallas_call(
            kernel,
            grid=(NT,),
            in_specs=[any_spec] * 6,
            out_specs=any_spec,
            out_shape=jax.ShapeDtypeStruct((S, D), BF),
            scratch_shapes=[pltpu.VMEM((3, D, D), BF),
                            pltpu.VMEM((N2, D, FC), BF),
                            pltpu.VMEM((N2, D, FC), BF),
                            pltpu.VMEM((N3, F, NO), BF),
                            pltpu.VMEM((N3, D, NO), BF),
                            pltpu.VMEM((NT, T, D), BF),
                            pltpu.VMEM((2, T, D), BF),
                            pltpu.VMEM((3, T, D), F32),
                            pltpu.VMEM((3, NC, T + HALO, 128), F32),
                            pltpu.VMEM((NC, R2, 128), F32),
                            pltpu.VMEM((T, D), BF),
                            pltpu.VMEM((N2, T, FC), BF),
                            pltpu.VMEM((N3, OSPLIT, T, OW), BF),
                            pltpu.SemaphoreType.DMA((NSEM,)),
                            pltpu.SemaphoreType.DMA((N3 * OSPLIT,))],
            compiler_params=pltpu.CompilerParams(dimension_semantics=("arbitrary",),
                                                 vmem_limit_bytes=110 * 1024 * 1024),
        )(x, wqkv, wo, w1, w3, w2)
    return run


_RUN = make(**{'XSPLIT':(128,128,128,128),'QSPLIT':(256,256,512),'OSPLIT':2,'PMODE':1})


@jax.jit
def pallas_recurrent_scan__sliding_local_dilated__glu_gated_swiglu__prompt_kernel(
    A_x: jax.Array,
    A_wqkv: jax.Array,
    A_wo: jax.Array,
    B_x: jax.Array,
    B_w1: jax.Array,
    B_w3: jax.Array,
    B_w2: jax.Array,
):
    del B_x
    out = _RUN(A_x.reshape(S, D), A_wqkv, A_wo, B_w1, B_w3, B_w2)
    return out.reshape(A_x.shape)
```

```python
import functools
import math
import jax
import jax.numpy as jnp
from jax import lax
import jax.experimental.pallas as pl
import jax.experimental.pallas.tpu as pltpu

S, D, F = 2048, 1024, 3584
H, DH, W, DIL = 32, 32, 8, 2
HALO = 16
NC = D // 128
BF = jnp.bfloat16
F32 = jnp.float32


def swap8(xs):
    xs = list(xs)
    lane = lax.broadcasted_iota(jnp.int32, xs[0].shape, 1)
    for b in range(3):
        s = 4 << b
        m = (lane & s) == 0
        for c in range(NC):
            if c & (1 << b):
                continue
            a, bb = xs[c], xs[c | (1 << b)]
            xs[c] = jnp.where(m, a, pltpu.roll(bb, s, 1))
            xs[c | (1 << b)] = jnp.where(m, pltpu.roll(a, 128 - s, 1), bb)
    return xs


def silu(x):
    a = 0.5 * x
    return a + a * jnp.tanh(a)


def ln_rows(x):
    m = jnp.mean(x, axis=-1, keepdims=True)
    xc = x - m
    var = jnp.mean(xc * xc, axis=-1, keepdims=True)
    return xc * lax.rsqrt(var + 1e-5)


def dot(a, b):
    return jnp.dot(a, b, preferred_element_type=F32)


def make(T=512, N2=2, N3=2, SB=16, RB=16, OB=32, chain=1, LNB=16, XSPLIT=(256, 256), QSPLIT=(256, 256, 512),
         OSPLIT=1, SUB=None, PMODE=0, UNIT=None, pvchain=0, lgchain=0):
    NT = S // T
    FC = F // N2
    NO = D // N3
    R2 = T // N2
    R3 = T // N3
    EXPC = (DH ** -0.5) * math.log2(math.e)
    assert sum(XSPLIT) == T and sum(QSPLIT) == D
    xoff = [sum(XSPLIT[:k]) for k in range(len(XSPLIT) + 1)]
    qoff = [sum(QSPLIT[:k]) for k in range(len(QSPLIT) + 1)]
    SX0 = 0
    SQ = SX0 + len(XSPLIT)
    SKV = SQ + len(QSPLIT)
    SW1 = SKV + 2
    SW3 = SW1 + N2
    SW2 = SW3 + N2
    SWO = SW2 + N3
    SX = SWO + N3
    NSEM = SX + NT - 1
    OW = NO // OSPLIT

    def kernel(x_hbm, wqkv_hbm, wo_hbm, w1_hbm, w3_hbm, w2_hbm, out_hbm,
               wq_s, w1_s, w3_s, w2_s, wo_s, x_s, xn_s, raw,
               qkv_s, o_s, ob_s, h_s, st_s, wsem, osem):
        i = pl.program_id(0)
        slot = i % 2
        q_s, k_s, v_s = qkv_s.at[0], qkv_s.at[1], qkv_s.at[2]

        def cp_x0(k):
            return pltpu.make_async_copy(x_hbm.at[xoff[k]:xoff[k + 1], :], x_s.at[0, xoff[k]:xoff[k + 1], :],
                                         wsem.at[SX0 + k])

        def cp_q(k):
            return pltpu.make_async_copy(wqkv_hbm.at[:, qoff[k]:qoff[k + 1]], wq_s.at[0, :, qoff[k]:qoff[k + 1]],
                                         wsem.at[SQ + k])

        def cp_kv(t):
            return pltpu.make_async_copy(wqkv_hbm.at[:, pl.ds(t * D, D)], wq_s.at[t], wsem.at[SKV + t - 1])

        def cp_w1(c):
            return pltpu.make_async_copy(w1_hbm.at[:, pl.ds(c * FC, FC)], w1_s.at[c], wsem.at[SW1 + c])

        def cp_w3(c):
            return pltpu.make_async_copy(w3_hbm.at[:, pl.ds(c * FC, FC)], w3_s.at[c], wsem.at[SW3 + c])

        def cp_w2(n):
            return pltpu.make_async_copy(w2_hbm.at[:, pl.ds(n * NO, NO)], w2_s.at[n], wsem.at[SW2 + n])

        def cp_wo(n):
            return pltpu.make_async_copy(wo_hbm.at[:, pl.ds(n * NO, NO)], wo_s.at[n], wsem.at[SWO + n])

        def cp_x(t):
            return pltpu.make_async_copy(x_hbm.at[pl.ds(t * T, T), :], x_s.at[t], wsem.at[SX + t - 1])

        def cp_out(n, p):
            return pltpu.make_async_copy(st_s.at[n, p], out_hbm.at[pl.ds(i * T, T), pl.ds(n * NO + p * OW, OW)],
                                         osem.at[n * OSPLIT + p])

        @pl.when(i == 0)
        def _():
            nx, nq = len(XSPLIT), len(QSPLIT)
            if PMODE == 0:
                for k in range(max(nx, nq)):
                    if k < nx:
                        cp_x0(k).start()
                    if k < nq:
                        cp_q(k).start()
            else:
                for k in range(nx):
                    cp_x0(k).start()
                for k in range(nq):
                    cp_q(k).start()
            for t in (1, 2):
                cp_kv(t).start()
            for c in range(N2):
                cp_w1(c).start()
                cp_w3(c).start()
            for n in range(N3):
                cp_w2(n).start()
                cp_wo(n).start()
            for t in range(1, NT):
                cp_x(t).start()
            k_s[:, T:T + HALO, :] = jnp.zeros((NC, HALO, 128), F32)
            v_s[:, T:T + HALO, :] = jnp.zeros((NC, HALO, 128), F32)
            if PMODE == 0:
                for k in range(nx):
                    cp_x0(k).wait()
                    for r0 in range(xoff[k], xoff[k + 1], 128):
                        xn_s[0, r0:r0 + 128, :] = ln_rows(x_s[0, r0:r0 + 128, :].astype(F32)).astype(BF)
                    if k == 0:
                        cp_q(0).wait()
                    raw[0, xoff[k]:xoff[k + 1], qoff[0]:qoff[1]] = dot(xn_s[0, xoff[k]:xoff[k + 1], :],
                                                                       wq_s[0, :, qoff[0]:qoff[1]])
                kq0 = 1
            else:
                for k in range(nx):
                    cp_x0(k).wait()
                    for r0 in range(xoff[k], xoff[k + 1], 128):
                        xn_s[0, r0:r0 + 128, :] = ln_rows(x_s[0, r0:r0 + 128, :].astype(F32)).astype(BF)
                kq0 = 0
            for k in range(kq0, nq):
                cp_q(k).wait()
                raw[0, :, qoff[k]:qoff[k + 1]] = dot(xn_s[0], wq_s[0, :, qoff[k]:qoff[k + 1]])

        def swap_rows(src, dst, base, nrows):
            for r0 in range(0, nrows, 2 * SB):
                ps = [pltpu.pack_elementwise(
                    [src[pl.ds(base + r0, SB), c * 128:(c + 1) * 128],
                     src[pl.ds(base + r0 + SB, SB), c * 128:(c + 1) * 128]], packed_dtype=BF) for c in range(NC)]
                ys = swap8(ps)
                for c in range(NC):
                    dst[c, pl.ds(HALO + base + r0, SB), :] = pltpu.unpack_elementwise(
                        ys[c], index=0, packed_dtype=BF, unpacked_dtype=F32)
                    dst[c, pl.ds(HALO + base + r0 + SB, SB), :] = pltpu.unpack_elementwise(
                        ys[c], index=1, packed_dtype=BF, unpacked_dtype=F32)

        k_s[:, 0:HALO, :] = k_s[:, T:T + HALO, :]
        v_s[:, 0:HALO, :] = v_s[:, T:T + HALO, :]

        def pb(t, carry):
            @pl.when(i == 0)
            def _():
                cp_kv(t).wait()

            raw[t] = dot(xn_s[slot], wq_s[t])
            return carry

        lax.fori_loop(jnp.where(i == 0, 1, 0), 3, pb, 0)

        def attn_group(base, r0, dep):
            rb = base + r0
            qs = [q_s[c, pl.ds(HALO + rb, RB), :] for c in range(NC)]
            if dep is not None:
                qs[0] = jnp.where(i < 0, dep, qs[0])
            lane = lax.broadcasted_iota(jnp.int32, (RB, 128), 1)
            b0 = (lane & 1) == 0
            b1 = (lane & 2) == 0
            logits = []
            for j in range(W):
                st = HALO + rb - DIL * j
                q0 = qs[0]
                if lgchain and j >= lgchain:
                    q0 = jnp.where(i < 0, logits[j - lgchain], q0)
                acc = q0 * k_s[0, pl.ds(st, RB), :]
                for c in range(1, NC):
                    acc = acc + qs[c] * k_s[c, pl.ds(st, RB), :]
                logits.append(acc)
            logits = [acc + jnp.where(b0, pltpu.roll(acc, 127, 1), pltpu.roll(acc, 1, 1)) for acc in logits]
            logits = [acc + jnp.where(b1, pltpu.roll(acc, 126, 1), pltpu.roll(acc, 2, 1)) for acc in logits]
            if r0 < HALO:
                row = i * T + rb + lax.broadcasted_iota(jnp.int32, (RB, 128), 0)
                logits = [logits[0]] + [jnp.where(row >= DIL * j, logits[j], -1e9) for j in range(1, W)]
            mx = logits[0]
            for j in range(1, W):
                mx = jnp.maximum(mx, logits[j])
            es = [jnp.exp2((l - mx) * EXPC) for l in logits]
            den = es[0]
            for j in range(1, W):
                den = den + es[j]
            inv = 1.0 / den
            ps = [e * inv for e in es]
            accs = []
            for c in range(NC):
                acc = None
                for j in range(W):
                    st = HALO + rb - DIL * j
                    pj = ps[j]
                    if j == 0 and pvchain and c >= pvchain:
                        pj = jnp.where(i < 0, accs[c - pvchain], pj)
                    t = pj * v_s[c, pl.ds(st, RB), :]
                    acc = t if acc is None else acc + t
                accs.append(acc)
                o_s[c, r0:r0 + RB, :] = acc
            return acc

        def p2(c, carry):
            @pl.when(i == 0)
            def _():
                cp_w1(c).wait()
                cp_w3(c).wait()

            base = pl.multiple_of(c * R2, R2)
            sub = SUB or FC
            for s0 in range(0, FC, sub):
                s1 = min(s0 + sub, FC)
                g = dot(xn_s[slot], w1_s[c, :, s0:s1])
                u = dot(xn_s[slot], w3_s[c, :, s0:s1])
                h_s[c, :, s0:s1] = (silu(g) * u).astype(BF)

            unit = UNIT or R2
            outs = []
            for u0 in range(0, R2, unit):
                for t in range(3):
                    swap_rows(raw.at[t], qkv_s.at[t], base + u0, unit)
                for r0 in range(u0, u0 + unit, RB):
                    dep = outs[-chain] if chain and len(outs) >= chain else None
                    outs.append(attn_group(base, r0, dep))
                for r0 in range(u0, u0 + unit, OB):
                    ts = [pltpu.bitcast(o_s[cc, r0:r0 + OB, :].astype(BF), jnp.uint32) for cc in range(NC)]
                    ts = swap8(ts)
                    for cc in range(NC):
                        ob_s[pl.ds(base + r0, OB), cc * 128:(cc + 1) * 128] = pltpu.bitcast(ts[cc], BF)
            return carry

        lax.fori_loop(0, N2, p2, 0)

        nxt = jnp.minimum(i + 1, NT - 1)

        def p3(n, carry):
            @pl.when(i == 0)
            def _():
                cp_w2(n).wait()
                cp_wo(n).wait()

            @pl.when(i > 0)
            def _():
                for p in range(OSPLIT):
                    cp_out(n, p).wait()

            @pl.when(jnp.logical_and(n == 0, i + 1 < NT))
            def _():
                cp_x(i + 1).wait()

            for p in range(OSPLIT):
                f = None
                for c in range(N2):
                    t = dot(h_s[c], w2_s[n, c * FC:(c + 1) * FC, p * OW:(p + 1) * OW])
                    f = t if f is None else f + t
                s = dot(ob_s[...], wo_s[n, :, p * OW:(p + 1) * OW])
                xr = x_s[i, :, pl.ds(pl.multiple_of(n * NO + p * OW, OW), OW)].astype(F32)
                st_s[n, p] = (xr + s * silu(f)).astype(BF)
                cp_out(n, p).start()

            rb = pl.multiple_of(n * R3, R3)
            prev = None
            for r0 in range(0, R3, LNB):
                xb = x_s[nxt, pl.ds(rb + r0, LNB), :].astype(F32)
                if prev is not None:
                    x0 = jnp.where(i < 0, prev, xb[:, 0:128])
                    xb = jnp.concatenate([x0, xb[:, 128:]], axis=1)
                y = ln_rows(xb)
                prev = y[:, 0:128]
                xn_s[1 - slot, pl.ds(rb + r0, LNB), :] = y.astype(BF)
            return carry

        lax.fori_loop(0, N3, p3, 0)

        @pl.when(i == NT - 1)
        def _():
            for n in range(N3):
                for p in range(OSPLIT):
                    cp_out(n, p).wait()

    any_spec = pl.BlockSpec(memory_space=pl.ANY)

    @jax.jit
    def run(x, wqkv, wo, w1, w3, w2):
        return pl.pallas_call(
            kernel,
            grid=(NT,),
            in_specs=[any_spec] * 6,
            out_specs=any_spec,
            out_shape=jax.ShapeDtypeStruct((S, D), BF),
            scratch_shapes=[pltpu.VMEM((3, D, D), BF),
                            pltpu.VMEM((N2, D, FC), BF),
                            pltpu.VMEM((N2, D, FC), BF),
                            pltpu.VMEM((N3, F, NO), BF),
                            pltpu.VMEM((N3, D, NO), BF),
                            pltpu.VMEM((NT, T, D), BF),
                            pltpu.VMEM((2, T, D), BF),
                            pltpu.VMEM((3, T, D), F32),
                            pltpu.VMEM((3, NC, T + HALO, 128), F32),
                            pltpu.VMEM((NC, R2, 128), F32),
                            pltpu.VMEM((T, D), BF),
                            pltpu.VMEM((N2, T, FC), BF),
                            pltpu.VMEM((N3, OSPLIT, T, OW), BF),
                            pltpu.SemaphoreType.DMA((NSEM,)),
                            pltpu.SemaphoreType.DMA((N3 * OSPLIT,))],
            compiler_params=pltpu.CompilerParams(dimension_semantics=("arbitrary",),
                                                 vmem_limit_bytes=110 * 1024 * 1024),
        )(x, wqkv, wo, w1, w3, w2)
    return run


_RUN = make(**{'XSPLIT':(128,128,128,128),'QSPLIT':(256,256,512),'PMODE':1,'pvchain':1,'UNIT':64,'OSPLIT':2})


@jax.jit
def pallas_recurrent_scan__sliding_local_dilated__glu_gated_swiglu__prompt_kernel(
    A_x: jax.Array,
    A_wqkv: jax.Array,
    A_wo: jax.Array,
    B_x: jax.Array,
    B_w1: jax.Array,
    B_w3: jax.Array,
    B_w2: jax.Array,
):
    del B_x
    out = _RUN(A_x.reshape(S, D), A_wqkv, A_wo, B_w1, B_w3, B_w2)
    return out.reshape(A_x.shape)
```

```python
import math

import jax
import jax.numpy as jnp
from jax import lax
import jax.experimental.pallas as pl
import jax.experimental.pallas.tpu as pltpu

S, D, F = 2048, 1024, 3584
H, DH, W, DIL = 32, 32, 8, 2
HALO = 16
NC = D // 128
BF = jnp.bfloat16
F32 = jnp.float32
U32 = jnp.uint32

T = 512
NT = S // T
N2 = 2
N3 = 2
FC = F // N2
NO = D // N3
R2 = T // N2
R3 = T // N3
SB = 16
RB = 16
OB = 32
UNIT = 64
LNB = 16
XSPLIT = (128, 128, 128, 128)
QSPLIT = (256, 256, 512)
OSPLIT = 2
OW = NO // OSPLIT
EXPC = (DH ** -0.5) * math.log2(math.e)

XOFF = [sum(XSPLIT[:k]) for k in range(len(XSPLIT) + 1)]
QOFF = [sum(QSPLIT[:k]) for k in range(len(QSPLIT) + 1)]
SX0 = 0
SQ = SX0 + len(XSPLIT)
SKV = SQ + len(QSPLIT)
SW1 = SKV + 2
SW3 = SW1 + N2
SW2 = SW3 + N2
SWO = SW2 + N3
SX = SWO + N3
NSEM = SX + NT - 1


def _swap8(xs):
    xs = list(xs)
    lane = lax.broadcasted_iota(jnp.int32, xs[0].shape, 1)
    for b in range(3):
        s = 4 << b
        m = (lane & s) == 0
        for c in range(NC):
            if c & (1 << b):
                continue
            lo, hi = xs[c], xs[c | (1 << b)]
            xs[c] = jnp.where(m, lo, pltpu.roll(hi, s, 1))
            xs[c | (1 << b)] = jnp.where(m, pltpu.roll(lo, 128 - s, 1), hi)
    return xs


def _silu(x):
    a = 0.5 * x
    return a + a * jnp.tanh(a)


def _layernorm(x):
    m = jnp.mean(x, axis=-1, keepdims=True)
    xc = x - m
    var = jnp.mean(xc * xc, axis=-1, keepdims=True)
    return xc * lax.rsqrt(var + 1e-5)


def _dot(a, b):
    return jnp.dot(a, b, preferred_element_type=F32)


def _kernel(x_hbm, wqkv_hbm, wo_hbm, w1_hbm, w3_hbm, w2_hbm, out_hbm,
            wq_s, w1_s, w3_s, w2_s, wo_s, x_s, xn_s, raw,
            qkv_s, o_s, ob_s, h_s, st_s, wsem, osem):
    i = pl.program_id(0)
    slot = i % 2
    q_s, k_s, v_s = qkv_s.at[0], qkv_s.at[1], qkv_s.at[2]

    def after(dep, x):
        return jnp.where(i < 0, dep, x)

    def cp_x0(k):
        return pltpu.make_async_copy(x_hbm.at[XOFF[k]:XOFF[k + 1], :], x_s.at[0, XOFF[k]:XOFF[k + 1], :],
                                     wsem.at[SX0 + k])

    def cp_q(k):
        return pltpu.make_async_copy(wqkv_hbm.at[:, QOFF[k]:QOFF[k + 1]], wq_s.at[0, :, QOFF[k]:QOFF[k + 1]],
                                     wsem.at[SQ + k])

    def cp_kv(t):
        return pltpu.make_async_copy(wqkv_hbm.at[:, pl.ds(t * D, D)], wq_s.at[t], wsem.at[SKV + t - 1])

    def cp_w1(c):
        return pltpu.make_async_copy(w1_hbm.at[:, pl.ds(c * FC, FC)], w1_s.at[c], wsem.at[SW1 + c])

    def cp_w3(c):
        return pltpu.make_async_copy(w3_hbm.at[:, pl.ds(c * FC, FC)], w3_s.at[c], wsem.at[SW3 + c])

    def cp_w2(n):
        return pltpu.make_async_copy(w2_hbm.at[:, pl.ds(n * NO, NO)], w2_s.at[n], wsem.at[SW2 + n])

    def cp_wo(n):
        return pltpu.make_async_copy(wo_hbm.at[:, pl.ds(n * NO, NO)], wo_s.at[n], wsem.at[SWO + n])

    def cp_x(t):
        return pltpu.make_async_copy(x_hbm.at[pl.ds(t * T, T), :], x_s.at[t], wsem.at[SX + t - 1])

    def cp_out(n, p):
        return pltpu.make_async_copy(st_s.at[n, p], out_hbm.at[pl.ds(i * T, T), pl.ds(n * NO + p * OW, OW)],
                                     osem.at[n * OSPLIT + p])

    @pl.when(i == 0)
    def _():
        for k in range(len(XSPLIT)):
            cp_x0(k).start()
        for k in range(len(QSPLIT)):
            cp_q(k).start()
        for t in (1, 2):
            cp_kv(t).start()
        for c in range(N2):
            cp_w1(c).start()
            cp_w3(c).start()
        for n in range(N3):
            cp_w2(n).start()
            cp_wo(n).start()
        for t in range(1, NT):
            cp_x(t).start()
        k_s[:, T:T + HALO, :] = jnp.zeros((NC, HALO, 128), F32)
        v_s[:, T:T + HALO, :] = jnp.zeros((NC, HALO, 128), F32)
        for k in range(len(XSPLIT)):
            cp_x0(k).wait()
            for r0 in range(XOFF[k], XOFF[k + 1], 128):
                xn_s[0, r0:r0 + 128, :] = _layernorm(x_s[0, r0:r0 + 128, :].astype(F32)).astype(BF)
        for k in range(len(QSPLIT)):
            cp_q(k).wait()
            raw[0, :, QOFF[k]:QOFF[k + 1]] = _dot(xn_s[0], wq_s[0, :, QOFF[k]:QOFF[k + 1]])

    k_s[:, 0:HALO, :] = k_s[:, T:T + HALO, :]
    v_s[:, 0:HALO, :] = v_s[:, T:T + HALO, :]

    def pb(t, carry):
        @pl.when(i == 0)
        def _():
            cp_kv(t).wait()

        raw[t] = _dot(xn_s[slot], wq_s[t])
        return carry

    lax.fori_loop(jnp.where(i == 0, 1, 0), 3, pb, 0)

    def swap_rows(src, dst, base, nrows):
        for r0 in range(0, nrows, 2 * SB):
            ps = [pltpu.pack_elementwise(
                [src[pl.ds(base + r0, SB), c * 128:(c + 1) * 128],
                 src[pl.ds(base + r0 + SB, SB), c * 128:(c + 1) * 128]], packed_dtype=BF) for c in range(NC)]
            ys = _swap8(ps)
            for c in range(NC):
                for half in range(2):
                    dst[c, pl.ds(HALO + base + r0 + half * SB, SB), :] = pltpu.unpack_elementwise(
                        ys[c], index=half, packed_dtype=BF, unpacked_dtype=F32)

    def attn_group(base, r0, dep):
        rb = base + r0
        qs = [q_s[c, pl.ds(HALO + rb, RB), :] for c in range(NC)]
        if dep is not None:
            qs[0] = after(dep, qs[0])
        lane = lax.broadcasted_iota(jnp.int32, (RB, 128), 1)
        b0 = (lane & 1) == 0
        b1 = (lane & 2) == 0
        logits = []
        for j in range(W):
            st = HALO + rb - DIL * j
            acc = qs[0] * k_s[0, pl.ds(st, RB), :]
            for c in range(1, NC):
                acc = acc + qs[c] * k_s[c, pl.ds(st, RB), :]
            logits.append(acc)
        logits = [a + jnp.where(b0, pltpu.roll(a, 127, 1), pltpu.roll(a, 1, 1)) for a in logits]
        logits = [a + jnp.where(b1, pltpu.roll(a, 126, 1), pltpu.roll(a, 2, 1)) for a in logits]
        if r0 < HALO:
            row = i * T + rb + lax.broadcasted_iota(jnp.int32, (RB, 128), 0)
            logits = [logits[0]] + [jnp.where(row >= DIL * j, logits[j], -1e9) for j in range(1, W)]
        mx = logits[0]
        for j in range(1, W):
            mx = jnp.maximum(mx, logits[j])
        es = [jnp.exp2((l - mx) * EXPC) for l in logits]
        den = es[0]
        for j in range(1, W):
            den = den + es[j]
        inv = 1.0 / den
        ps = [e * inv for e in es]
        acc = None
        for c in range(NC):
            p0 = ps[0] if acc is None else after(acc, ps[0])
            acc = p0 * v_s[c, pl.ds(HALO + rb, RB), :]
            for j in range(1, W):
                acc = acc + ps[j] * v_s[c, pl.ds(HALO + rb - DIL * j, RB), :]
            o_s[c, r0:r0 + RB, :] = acc
        return acc

    def p2(c, carry):
        @pl.when(i == 0)
        def _():
            cp_w1(c).wait()
            cp_w3(c).wait()

        base = pl.multiple_of(c * R2, R2)
        g = _dot(xn_s[slot], w1_s[c])
        u = _dot(xn_s[slot], w3_s[c])
        h_s[c] = (_silu(g) * u).astype(BF)

        dep = None
        for u0 in range(0, R2, UNIT):
            for t in range(3):
                swap_rows(raw.at[t], qkv_s.at[t], base + u0, UNIT)
            for r0 in range(u0, u0 + UNIT, RB):
                dep = attn_group(base, r0, dep)
            for r0 in range(u0, u0 + UNIT, OB):
                ts = [pltpu.bitcast(o_s[cc, r0:r0 + OB, :].astype(BF), U32) for cc in range(NC)]
                ts = _swap8(ts)
                for cc in range(NC):
                    ob_s[pl.ds(base + r0, OB), cc * 128:(cc + 1) * 128] = pltpu.bitcast(ts[cc], BF)
        return carry

    lax.fori_loop(0, N2, p2, 0)

    nxt = jnp.minimum(i + 1, NT - 1)

    def p3(n, carry):
        @pl.when(i == 0)
        def _():
            cp_w2(n).wait()
            cp_wo(n).wait()

        @pl.when(i > 0)
        def _():
            for p in range(OSPLIT):
                cp_out(n, p).wait()

        @pl.when(jnp.logical_and(n == 0, i + 1 < NT))
        def _():
            cp_x(i + 1).wait()

        for p in range(OSPLIT):
            f = _dot(h_s[0], w2_s[n, 0:FC, p * OW:(p + 1) * OW])
            for c in range(1, N2):
                f = f + _dot(h_s[c], w2_s[n, c * FC:(c + 1) * FC, p * OW:(p + 1) * OW])
            s = _dot(ob_s[...], wo_s[n, :, p * OW:(p + 1) * OW])
            xr = x_s[i, :, pl.ds(pl.multiple_of(n * NO + p * OW, OW), OW)].astype(F32)
            st_s[n, p] = (xr + s * _silu(f)).astype(BF)
            cp_out(n, p).start()

        rb = pl.multiple_of(n * R3, R3)
        prev = None
        for r0 in range(0, R3, LNB):
            xb = x_s[nxt, pl.ds(rb + r0, LNB), :].astype(F32)
            if prev is not None:
                xb = jnp.concatenate([after(prev, xb[:, 0:128]), xb[:, 128:]], axis=1)
            y = _layernorm(xb)
            prev = y[:, 0:128]
            xn_s[1 - slot, pl.ds(rb + r0, LNB), :] = y.astype(BF)
        return carry

    lax.fori_loop(0, N3, p3, 0)

    @pl.when(i == NT - 1)
    def _():
        for n in range(N3):
            for p in range(OSPLIT):
                cp_out(n, p).wait()


@jax.jit
def pallas_recurrent_scan__sliding_local_dilated__glu_gated_swiglu__prompt_kernel(
    A_x: jax.Array,
    A_wqkv: jax.Array,
    A_wo: jax.Array,
    B_x: jax.Array,
    B_w1: jax.Array,
    B_w3: jax.Array,
    B_w2: jax.Array,
):
    del B_x
    any_spec = pl.BlockSpec(memory_space=pl.ANY)
    out = pl.pallas_call(
        _kernel,
        grid=(NT,),
        in_specs=[any_spec] * 6,
        out_specs=any_spec,
        out_shape=jax.ShapeDtypeStruct((S, D), BF),
        scratch_shapes=[pltpu.VMEM((3, D, D), BF),
                        pltpu.VMEM((N2, D, FC), BF),
                        pltpu.VMEM((N2, D, FC), BF),
                        pltpu.VMEM((N3, F, NO), BF),
                        pltpu.VMEM((N3, D, NO), BF),
                        pltpu.VMEM((NT, T, D), BF),
                        pltpu.VMEM((2, T, D), BF),
                        pltpu.VMEM((3, T, D), F32),
                        pltpu.VMEM((3, NC, T + HALO, 128), F32),
                        pltpu.VMEM((NC, R2, 128), F32),
                        pltpu.VMEM((T, D), BF),
                        pltpu.VMEM((N2, T, FC), BF),
                        pltpu.VMEM((N3, OSPLIT, T, OW), BF),
                        pltpu.SemaphoreType.DMA((NSEM,)),
                        pltpu.SemaphoreType.DMA((N3 * OSPLIT,))],
        compiler_params=pltpu.CompilerParams(dimension_semantics=("arbitrary",),
                                             vmem_limit_bytes=110 * 1024 * 1024),
    )(A_x.reshape(S, D), A_wqkv, A_wo, B_w1, B_w3, B_w2)
    return out.reshape(A_x.shape)
```

```python
import math

import jax
import jax.numpy as jnp
from jax import lax
import jax.experimental.pallas as pl
import jax.experimental.pallas.tpu as pltpu

S, D, F = 2048, 1024, 3584
H, DH, W, DIL = 32, 32, 8, 2
HALO = 16
NC = D // 128
BF = jnp.bfloat16
F32 = jnp.float32
U32 = jnp.uint32

T1 = 512
T2 = 256
N1 = S // T1
N2 = S // T2
LH = T1 // 2
SUB = 1792
SB = 8
RB = 16
OB = 32
LNB = 16
XP = 128
NXP = T1 // XP
HR = 3 * XP
QOFF = (0, 256, 512, 1024)
OSPLIT = 4
OW = D // OSPLIT
EXPC = (DH ** -0.5) * math.log2(math.e)

SX0 = 0
SQ = SX0 + NXP
SKV = SQ + len(QOFF) - 1
SX = SKV + 2
SW = SX + 2 * (N1 - 1)
NSEM = SW + 4


def _swap8(xs):
    xs = list(xs)
    lane = lax.broadcasted_iota(jnp.int32, xs[0].shape, 1)
    for b in range(3):
        s = 4 << b
        m = (lane & s) == 0
        for c in range(NC):
            if c & (1 << b):
                continue
            lo, hi = xs[c], xs[c | (1 << b)]
            xs[c] = jnp.where(m, lo, pltpu.roll(hi, s, 1))
            xs[c | (1 << b)] = jnp.where(m, pltpu.roll(lo, 128 - s, 1), hi)
    return xs


def _silu(x):
    a = 0.5 * x
    return a + a * jnp.tanh(a)


def _layernorm(x):
    m = jnp.mean(x, axis=-1, keepdims=True)
    xc = x - m
    var = jnp.mean(xc * xc, axis=-1, keepdims=True)
    return xc * lax.rsqrt(var + 1e-5)


def _dot(a, b):
    return jnp.dot(a, b, preferred_element_type=F32)


def _after(idx, dep, x):
    return jnp.where(idx < 0, dep, x)


def _kernel(x_hbm, wqkv_hbm, wo_hbm, w1_hbm, w3_hbm, w2_hbm, out_hbm,
            wq_s, w1_s, w3_s, w2_s, wo_s, x_s, xn_s, raw,
            qkv_s, o_s, ob_s, h_s, st_s, wsem, osem):

    def cp_x0(k):
        return pltpu.make_async_copy(x_hbm.at[k * XP:(k + 1) * XP, :], x_s.at[0, k * XP:(k + 1) * XP, :],
                                     wsem.at[SX0 + k])

    def cp_q(k):
        return pltpu.make_async_copy(wqkv_hbm.at[:, QOFF[k]:QOFF[k + 1]], wq_s.at[0, :, QOFF[k]:QOFF[k + 1]],
                                     wsem.at[SQ + k])

    def cp_kv(t):
        return pltpu.make_async_copy(wqkv_hbm.at[:, pl.ds(t * D, D)], wq_s.at[t], wsem.at[SKV + t - 1])

    def cp_x(rb, h):
        return pltpu.make_async_copy(x_hbm.at[pl.ds(rb * T1 + h * LH, LH), :], x_s.at[rb, pl.ds(h * LH, LH), :],
                                     wsem.at[SX + 2 * (rb - 1) + h])

    def cp_w(k):
        src, dst = ((w1_hbm, w1_s), (w3_hbm, w3_s), (w2_hbm, w2_s), (wo_hbm, wo_s))[k]
        return pltpu.make_async_copy(src, dst, wsem.at[SW + k])

    def cp_out(b, p):
        slot = b % 2
        return pltpu.make_async_copy(st_s.at[slot, p], out_hbm.at[pl.ds(b * T2, T2), p * OW:(p + 1) * OW],
                                     osem.at[slot * OSPLIT + p])

    def ln0(k):
        xn_s[0, k * XP:(k + 1) * XP, :] = _layernorm(x_s[0, k * XP:(k + 1) * XP, :].astype(F32)).astype(BF)

    def qdot(r0, r1, c0, c1):
        raw[0, r0:r1, c0:c1] = _dot(xn_s[0, r0:r1, :], wq_s[0, :, c0:c1])

    nfirst = HR // XP
    for k in range(nfirst):
        cp_x0(k).start()
    cp_q(0).start()
    cp_q(1).start()
    for k in range(nfirst, NXP):
        cp_x0(k).start()
    cp_q(2).start()
    cp_kv(1).start()
    cp_x(1, 1).start()
    cp_kv(2).start()
    cp_x(1, 0).start()
    for rb in range(2, N1):
        cp_x(rb, 0).start()
        cp_x(rb, 1).start()
    for k in range(4):
        cp_w(k).start()
    qkv_s[1:3, :, T2:T2 + HALO, :] = jnp.zeros((2, NC, HALO, 128), F32)
    for k in range(nfirst):
        cp_x0(k).wait()
        ln0(k)
    cp_q(0).wait()
    qdot(0, HR, QOFF[0], QOFF[1])
    cp_q(1).wait()
    for k in range(nfirst, NXP):
        cp_x0(k).wait()
    qdot(0, HR, QOFF[1], QOFF[2])
    for k in range(nfirst, NXP):
        ln0(k)
    qdot(HR, T1, QOFF[0], QOFF[2])
    cp_q(2).wait()
    qdot(0, T1, QOFF[2], QOFF[3])

    def p1(it, carry):
        rb = it // 3
        t = it % 3

        @pl.when(jnp.logical_and(rb == 0, t > 0))
        def _():
            cp_kv(t).wait()

        @pl.when(jnp.logical_and(jnp.logical_or(t < 2, rb == 0), rb + 1 < N1))
        def _():
            cp_x(rb + 1, t % 2).wait()

        raw[t, pl.ds(pl.multiple_of(rb * T1, T1), T1), :] = _dot(xn_s[rb], wq_s[t])

        nb = jnp.minimum(rb + 1, N1 - 1)
        lb = pl.multiple_of((t % 2) * LH, LH)
        prev = None
        for r0 in range(0, LH, LNB):
            xb = x_s[nb, pl.ds(lb + r0, LNB), :].astype(F32)
            if prev is not None:
                xb = jnp.concatenate([_after(it, prev, xb[:, 0:128]), xb[:, 128:]], axis=1)
            y = _layernorm(xb)
            prev = y[:, 0:128]
            xn_s[nb, pl.ds(lb + r0, LNB), :] = y.astype(BF)
        return carry

    lax.fori_loop(1, 3 * N1, p1, 0)
    for k in range(4):
        cp_w(k).wait()

    def swap_rows(t, row0):
        for r0 in range(0, T2, 2 * SB):
            ps = [pltpu.pack_elementwise(
                [raw[t, pl.ds(row0 + r0, SB), c * 128:(c + 1) * 128],
                 raw[t, pl.ds(row0 + r0 + SB, SB), c * 128:(c + 1) * 128]], packed_dtype=BF) for c in range(NC)]
            ys = _swap8(ps)
            for c in range(NC):
                for half in range(2):
                    a = HALO + r0 + half * SB
                    qkv_s[t, c, a:a + SB, :] = pltpu.unpack_elementwise(
                        ys[c], index=half, packed_dtype=BF, unpacked_dtype=F32)

    def attn_group(b, r0, dep):
        qs = [qkv_s[0, c, HALO + r0:HALO + r0 + RB, :] for c in range(NC)]
        if dep is not None:
            qs[0] = _after(b, dep, qs[0])
        lane = lax.broadcasted_iota(jnp.int32, (RB, 128), 1)
        b0 = (lane & 1) == 0
        b1 = (lane & 2) == 0
        logits = []
        for j in range(W):
            st = HALO + r0 - DIL * j
            acc = qs[0] * qkv_s[1, 0, st:st + RB, :]
            for c in range(1, NC):
                acc = acc + qs[c] * qkv_s[1, c, st:st + RB, :]
            logits.append(acc)
        logits = [a + jnp.where(b0, pltpu.roll(a, 127, 1), pltpu.roll(a, 1, 1)) for a in logits]
        logits = [a + jnp.where(b1, pltpu.roll(a, 126, 1), pltpu.roll(a, 2, 1)) for a in logits]
        if r0 < HALO:
            row = b * T2 + r0 + lax.broadcasted_iota(jnp.int32, (RB, 128), 0)
            logits = [logits[0]] + [jnp.where(row >= DIL * j, logits[j], -1e9) for j in range(1, W)]
        mx = logits[0]
        for j in range(1, W):
            mx = jnp.maximum(mx, logits[j])
        es = [jnp.exp2((l - mx) * EXPC) for l in logits]
        den = es[0]
        for j in range(1, W):
            den = den + es[j]
        inv = 1.0 / den
        ps = [e * inv for e in es]
        acc = None
        for c in range(NC):
            p0 = ps[0] if acc is None else _after(b, acc, ps[0])
            acc = p0 * qkv_s[2, c, HALO + r0:HALO + r0 + RB, :]
            for j in range(1, W):
                st = HALO + r0 - DIL * j
                acc = acc + ps[j] * qkv_s[2, c, st:st + RB, :]
            o_s[c, r0:r0 + RB, :] = acc
        return acc

    def p2(b, carry):
        slot = b % 2

        @pl.when(b >= 2)
        def _():
            for p in range(OSPLIT):
                cp_out(b - 2, p).wait()

        row0 = pl.multiple_of(b * T2, T2)
        blk = b // (T1 // T2)
        off = pl.multiple_of((b % (T1 // T2)) * T2, T2)
        qkv_s[1:3, :, 0:HALO, :] = qkv_s[1:3, :, T2:T2 + HALO, :]

        xn = xn_s[blk, pl.ds(off, T2), :]
        for s0 in range(0, F, SUB):
            g = _dot(xn, w1_s[:, s0:s0 + SUB])
            u = _dot(xn, w3_s[:, s0:s0 + SUB])
            h_s[:, s0:s0 + SUB] = (_silu(g) * u).astype(BF)

        for t in range(3):
            swap_rows(t, row0)
        dep = None
        for r0 in range(0, T2, RB):
            dep = attn_group(b, r0, dep)
        for r0 in range(0, T2, OB):
            ts = [pltpu.bitcast(o_s[c, r0:r0 + OB, :].astype(BF), U32) for c in range(NC)]
            ts = _swap8(ts)
            for c in range(NC):
                ob_s[r0:r0 + OB, c * 128:(c + 1) * 128] = pltpu.bitcast(ts[c], BF)

        for p in range(OSPLIT):
            f = _dot(h_s[...], w2_s[:, p * OW:(p + 1) * OW])
            s = _dot(ob_s[...], wo_s[:, p * OW:(p + 1) * OW])
            xr = x_s[blk, pl.ds(off, T2), p * OW:(p + 1) * OW].astype(F32)
            st_s[slot, p] = (xr + s * _silu(f)).astype(BF)
            cp_out(b, p).start()
        return carry

    lax.fori_loop(0, N2, p2, 0)
    for b in (N2 - 2, N2 - 1):
        for p in range(OSPLIT):
            cp_out(b, p).wait()


@jax.jit
def pallas_recurrent_scan__sliding_local_dilated__glu_gated_swiglu__prompt_kernel(
    A_x: jax.Array,
    A_wqkv: jax.Array,
    A_wo: jax.Array,
    B_x: jax.Array,
    B_w1: jax.Array,
    B_w3: jax.Array,
    B_w2: jax.Array,
):
    del B_x
    any_spec = pl.BlockSpec(memory_space=pl.ANY)
    out = pl.pallas_call(
        _kernel,
        in_specs=[any_spec] * 6,
        out_specs=any_spec,
        out_shape=jax.ShapeDtypeStruct((S, D), BF),
        scratch_shapes=[pltpu.VMEM((3, D, D), BF),
                        pltpu.VMEM((D, F), BF),
                        pltpu.VMEM((D, F), BF),
                        pltpu.VMEM((F, D), BF),
                        pltpu.VMEM((D, D), BF),
                        pltpu.VMEM((N1, T1, D), BF),
                        pltpu.VMEM((N1, T1, D), BF),
                        pltpu.VMEM((3, S, D), F32),
                        pltpu.VMEM((3, NC, T2 + HALO, 128), F32),
                        pltpu.VMEM((NC, T2, 128), F32),
                        pltpu.VMEM((T2, D), BF),
                        pltpu.VMEM((T2, F), BF),
                        pltpu.VMEM((2, OSPLIT, T2, OW), BF),
                        pltpu.SemaphoreType.DMA((NSEM,)),
                        pltpu.SemaphoreType.DMA((2 * OSPLIT,))],
        compiler_params=pltpu.CompilerParams(vmem_limit_bytes=110 * 1024 * 1024),
    )(A_x.reshape(S, D), A_wqkv, A_wo, B_w1, B_w3, B_w2)
    return out.reshape(A_x.shape)
```

```python
import math

import jax
import jax.numpy as jnp
from jax import lax
import jax.experimental.pallas as pl
import jax.experimental.pallas.tpu as pltpu

S, D, F = 2048, 1024, 3584
H, DH, W, DIL = 32, 32, 8, 2
HALO = 16
NC = D // 128
BF = jnp.bfloat16
F32 = jnp.float32
U32 = jnp.uint32

T1 = 512
T2 = 256
N1 = S // T1
N2 = S // T2
LH = T1 // 2
SUB = 1792
SB = 8
RB = 16
OB = 32
LNB = 16
XP = 128
NXP = T1 // XP
HR = 3 * XP
QOFF = (0, 256, 512, 1024, 1536)
HW = 3 * D // 2
OSPLIT = 4
OW = D // OSPLIT
EXPC = (DH ** -0.5) * math.log2(math.e)

SX0 = 0
SQ = SX0 + NXP
SKV = SQ + len(QOFF) - 1
SX = SKV + 1
SW = SX + 2 * (N1 - 1)
NSEM = SW + 4


def _swap8(xs):
    xs = list(xs)
    lane = lax.broadcasted_iota(jnp.int32, xs[0].shape, 1)
    for b in range(3):
        s = 4 << b
        m = (lane & s) == 0
        for c in range(NC):
            if c & (1 << b):
                continue
            lo, hi = xs[c], xs[c | (1 << b)]
            xs[c] = jnp.where(m, lo, pltpu.roll(hi, s, 1))
            xs[c | (1 << b)] = jnp.where(m, pltpu.roll(lo, 128 - s, 1), hi)
    return xs


def _silu(x):
    a = 0.5 * x
    return a + a * jnp.tanh(a)


def _layernorm(x):
    m = jnp.mean(x, axis=-1, keepdims=True)
    xc = x - m
    var = jnp.mean(xc * xc, axis=-1, keepdims=True)
    return xc * lax.rsqrt(var + 1e-5)


def _dot(a, b):
    return jnp.dot(a, b, preferred_element_type=F32)


def _after(idx, dep, x):
    return jnp.where(idx < 0, dep, x)


def _kernel(x_hbm, wqkv_hbm, wo_hbm, w1_hbm, w3_hbm, w2_hbm, out_hbm,
            wq_s, w1_s, w3_s, w2_s, wo_s, x_s, xn_s, raw,
            qkv_s, o_s, ob_s, h_s, st_s, wsem, osem):

    def cp_x0(k):
        return pltpu.make_async_copy(x_hbm.at[k * XP:(k + 1) * XP, :], x_s.at[0, k * XP:(k + 1) * XP, :],
                                     wsem.at[SX0 + k])

    def cp_q(k):
        return pltpu.make_async_copy(wqkv_hbm.at[:, QOFF[k]:QOFF[k + 1]], wq_s.at[0, :, QOFF[k]:QOFF[k + 1]],
                                     wsem.at[SQ + k])

    def cp_h1():
        return pltpu.make_async_copy(wqkv_hbm.at[:, HW:2 * HW], wq_s.at[1], wsem.at[SKV])

    def cp_x(rb, h):
        return pltpu.make_async_copy(x_hbm.at[pl.ds(rb * T1 + h * LH, LH), :], x_s.at[rb, pl.ds(h * LH, LH), :],
                                     wsem.at[SX + 2 * (rb - 1) + h])

    def cp_w(k):
        src, dst = ((w1_hbm, w1_s), (w3_hbm, w3_s), (w2_hbm, w2_s), (wo_hbm, wo_s))[k]
        return pltpu.make_async_copy(src, dst, wsem.at[SW + k])

    def cp_out(b, p):
        slot = b % 2
        return pltpu.make_async_copy(st_s.at[slot, p], out_hbm.at[pl.ds(b * T2, T2), p * OW:(p + 1) * OW],
                                     osem.at[slot * OSPLIT + p])

    def ln_half(idx, nb, h):
        lb = h * LH if idx is None else pl.multiple_of(h * LH, LH)
        prev = None
        for r0 in range(0, LH, LNB):
            xb = x_s[nb, pl.ds(lb + r0, LNB), :].astype(F32)
            if prev is not None and idx is not None:
                xb = jnp.concatenate([_after(idx, prev, xb[:, 0:128]), xb[:, 128:]], axis=1)
            y = _layernorm(xb)
            prev = y[:, 0:128]
            xn_s[nb, pl.ds(lb + r0, LNB), :] = y.astype(BF)

    def ln0(k):
        xn_s[0, k * XP:(k + 1) * XP, :] = _layernorm(x_s[0, k * XP:(k + 1) * XP, :].astype(F32)).astype(BF)

    def qdot(r0, r1, c0, c1):
        raw[0, r0:r1, c0:c1] = _dot(xn_s[0, r0:r1, :], wq_s[0, :, c0:c1])

    nfirst = HR // XP
    for k in range(nfirst):
        cp_x0(k).start()
    cp_q(0).start()
    cp_q(1).start()
    for k in range(nfirst, NXP):
        cp_x0(k).start()
    cp_q(2).start()
    cp_x(1, 0).start()
    cp_q(3).start()
    cp_x(1, 1).start()
    cp_h1().start()
    for rb in range(2, N1):
        cp_x(rb, 0).start()
        cp_x(rb, 1).start()
    for k in range(4):
        cp_w(k).start()
    qkv_s[1:3, :, T2:T2 + HALO, :] = jnp.zeros((2, NC, HALO, 128), F32)
    for k in range(nfirst):
        cp_x0(k).wait()
        ln0(k)
    cp_q(0).wait()
    qdot(0, HR, QOFF[0], QOFF[1])
    cp_q(1).wait()
    for k in range(nfirst, NXP):
        cp_x0(k).wait()
    qdot(0, HR, QOFF[1], QOFF[2])
    for k in range(nfirst, NXP):
        ln0(k)
    qdot(HR, T1, QOFF[0], QOFF[2])
    cp_q(2).wait()
    qdot(0, T1, QOFF[2], QOFF[3])
    cp_q(3).wait()
    cp_x(1, 0).wait()
    qdot(0, T1, QOFF[3], QOFF[4])
    ln_half(None, 1, 0)

    def p1(it, carry):
        rb = it // 2
        t = it % 2

        @pl.when(it == 1)
        def _():
            cp_h1().wait()

        @pl.when(rb + 1 < N1)
        def _():
            cp_x(rb + 1, t).wait()

        raw[t, pl.ds(pl.multiple_of(rb * T1, T1), T1), :] = _dot(xn_s[rb], wq_s[t])
        ln_half(it, jnp.minimum(rb + 1, N1 - 1), t)
        return carry

    lax.fori_loop(1, 2 * N1, p1, 0)
    for k in range(4):
        cp_w(k).wait()

    def swap_rows(t, row0):
        def src(r, c):
            col = t * D + c * 128
            return raw[col // HW, pl.ds(row0 + r, SB), col % HW:col % HW + 128]

        for r0 in range(0, T2, 2 * SB):
            ps = [pltpu.pack_elementwise([src(r0, c), src(r0 + SB, c)], packed_dtype=BF) for c in range(NC)]
            ys = _swap8(ps)
            for c in range(NC):
                for half in range(2):
                    a = HALO + r0 + half * SB
                    qkv_s[t, c, a:a + SB, :] = pltpu.unpack_elementwise(
                        ys[c], index=half, packed_dtype=BF, unpacked_dtype=F32)

    def attn_group(b, r0, dep):
        qs = [qkv_s[0, c, HALO + r0:HALO + r0 + RB, :] for c in range(NC)]
        if dep is not None:
            qs[0] = _after(b, dep, qs[0])
        lane = lax.broadcasted_iota(jnp.int32, (RB, 128), 1)
        b0 = (lane & 1) == 0
        b1 = (lane & 2) == 0
        logits = []
        for j in range(W):
            st = HALO + r0 - DIL * j
            acc = qs[0] * qkv_s[1, 0, st:st + RB, :]
            for c in range(1, NC):
                acc = acc + qs[c] * qkv_s[1, c, st:st + RB, :]
            logits.append(acc)
        logits = [a + jnp.where(b0, pltpu.roll(a, 127, 1), pltpu.roll(a, 1, 1)) for a in logits]
        logits = [a + jnp.where(b1, pltpu.roll(a, 126, 1), pltpu.roll(a, 2, 1)) for a in logits]
        if r0 < HALO:
            row = b * T2 + r0 + lax.broadcasted_iota(jnp.int32, (RB, 128), 0)
            logits = [logits[0]] + [jnp.where(row >= DIL * j, logits[j], -1e9) for j in range(1, W)]
        mx = logits[0]
        for j in range(1, W):
            mx = jnp.maximum(mx, logits[j])
        es = [jnp.exp2((l - mx) * EXPC) for l in logits]
        den = es[0]
        for j in range(1, W):
            den = den + es[j]
        inv = 1.0 / den
        ps = [e * inv for e in es]
        acc = None
        for c in range(NC):
            p0 = ps[0] if acc is None else _after(b, acc, ps[0])
            acc = p0 * qkv_s[2, c, HALO + r0:HALO + r0 + RB, :]
            for j in range(1, W):
                st = HALO + r0 - DIL * j
                acc = acc + ps[j] * qkv_s[2, c, st:st + RB, :]
            o_s[c, r0:r0 + RB, :] = acc
        return acc

    def p2(b, carry):
        slot = b % 2

        @pl.when(b >= 2)
        def _():
            for p in range(OSPLIT):
                cp_out(b - 2, p).wait()

        row0 = pl.multiple_of(b * T2, T2)
        blk = b // (T1 // T2)
        off = pl.multiple_of((b % (T1 // T2)) * T2, T2)
        qkv_s[1:3, :, 0:HALO, :] = qkv_s[1:3, :, T2:T2 + HALO, :]

        xn = xn_s[blk, pl.ds(off, T2), :]
        for s0 in range(0, F, SUB):
            g = _dot(xn, w1_s[:, s0:s0 + SUB])
            u = _dot(xn, w3_s[:, s0:s0 + SUB])
            h_s[:, s0:s0 + SUB] = (_silu(g) * u).astype(BF)

        for t in range(3):
            swap_rows(t, row0)
        dep = None
        for r0 in range(0, T2, RB):
            dep = attn_group(b, r0, dep)
        for r0 in range(0, T2, OB):
            ts = [pltpu.bitcast(o_s[c, r0:r0 + OB, :].astype(BF), U32) for c in range(NC)]
            ts = _swap8(ts)
            for c in range(NC):
                ob_s[r0:r0 + OB, c * 128:(c + 1) * 128] = pltpu.bitcast(ts[c], BF)

        for p in range(OSPLIT):
            f = _dot(h_s[...], w2_s[:, p * OW:(p + 1) * OW])
            s = _dot(ob_s[...], wo_s[:, p * OW:(p + 1) * OW])
            xr = x_s[blk, pl.ds(off, T2), p * OW:(p + 1) * OW].astype(F32)
            st_s[slot, p] = (xr + s * _silu(f)).astype(BF)
            cp_out(b, p).start()
        return carry

    lax.fori_loop(0, N2, p2, 0)
    for b in (N2 - 2, N2 - 1):
        for p in range(OSPLIT):
            cp_out(b, p).wait()


@jax.jit
def pallas_recurrent_scan__sliding_local_dilated__glu_gated_swiglu__prompt_kernel(
    A_x: jax.Array,
    A_wqkv: jax.Array,
    A_wo: jax.Array,
    B_x: jax.Array,
    B_w1: jax.Array,
    B_w3: jax.Array,
    B_w2: jax.Array,
):
    del B_x
    any_spec = pl.BlockSpec(memory_space=pl.ANY)
    out = pl.pallas_call(
        _kernel,
        in_specs=[any_spec] * 6,
        out_specs=any_spec,
        out_shape=jax.ShapeDtypeStruct((S, D), BF),
        scratch_shapes=[pltpu.VMEM((2, D, HW), BF),
                        pltpu.VMEM((D, F), BF),
                        pltpu.VMEM((D, F), BF),
                        pltpu.VMEM((F, D), BF),
                        pltpu.VMEM((D, D), BF),
                        pltpu.VMEM((N1, T1, D), BF),
                        pltpu.VMEM((N1, T1, D), BF),
                        pltpu.VMEM((2, S, HW), F32),
                        pltpu.VMEM((3, NC, T2 + HALO, 128), F32),
                        pltpu.VMEM((NC, T2, 128), F32),
                        pltpu.VMEM((T2, D), BF),
                        pltpu.VMEM((T2, F), BF),
                        pltpu.VMEM((2, OSPLIT, T2, OW), BF),
                        pltpu.SemaphoreType.DMA((NSEM,)),
                        pltpu.SemaphoreType.DMA((2 * OSPLIT,))],
        compiler_params=pltpu.CompilerParams(vmem_limit_bytes=110 * 1024 * 1024),
    )(A_x.reshape(S, D), A_wqkv, A_wo, B_w1, B_w3, B_w2)
    return out.reshape(A_x.shape)
```
